```python
import jax
import jax.numpy as jnp

def _softmax(x, axis=-1):
    return jax.nn.softmax(x, axis=axis)
def _gelu(x):
    return jax.nn.gelu(x, approximate=True)
def _silu(x):
    return jax.nn.silu(x)
def _sigmoid(x):
    return jax.nn.sigmoid(x)
def _layernorm(x, axis=-1, eps=1e-5):
    m = jnp.mean(x, axis=axis, keepdims=True)
    v = jnp.var(x, axis=axis, keepdims=True)
    return (x - m) / jnp.sqrt(v + eps)
def _scatter_add(tgt, idx, src, axis=0):
    return tgt.at[idx].add(src)
def _segment_sum(src, seg, n):
    return jax.ops.segment_sum(src, seg, n)
class _Rng:
    def __init__(self, key):
        self._k = key
    def _next(self):
        self._k, sub = jax.random.split(self._k)
        return sub
    def normal(self, shape):
        return jax.random.normal(self._next(), shape, dtype=jnp.bfloat16)
    def randint(self, lo, hi, shape):
        return jax.random.randint(self._next(), shape, lo, hi, dtype=jnp.int32)
    def uniform(self, shape, lo=0.0, hi=1.0):
        return jax.random.uniform(self._next(), shape, jnp.bfloat16, lo, hi)
    def permutation(self, n):
        return jax.random.permutation(self._next(), n)


kernel_name = 'interleave_layers__sliding_local_dilated__mixer_token_mlp__prompt'

def setup_inputs():
    _rng = _Rng(jax.random.key(int.from_bytes(__import__("os").urandom(4), "little")))
    _w = (lambda a: (lambda t: t.astype(jnp.bfloat16) if jnp.issubdtype(t.dtype, jnp.floating) else t)(jnp.asarray(a)))
    def _A_setup():
        B, S, D = 1, 2048, 1024
        return {
            "x": _w((lambda *s: _rng.normal(s) * 0.05)(B, S, D)),
            "wqkv": _w((lambda *s: _rng.normal(s) * 0.05)(D, 3 * D)),
            "wo": _w((lambda *s: _rng.normal(s) * 0.05)(D, D)),
        }
    _A_in = _A_setup()

    def _B_setup():
        B, S, D, F = 1, 2048, 1024, 3584
        return {
            "x": _w((lambda *s: _rng.normal(s) * 0.05)(B, S, D)),
            "w1": _w((lambda *s: _rng.normal(s) * 0.05)(S, F) * (S ** -0.5)),
            "b1": _w((lambda *s: _rng.normal(s) * 0.05)(F) * 0.02),
            "w2": _w((lambda *s: _rng.normal(s) * 0.05)(F, S) * (F ** -0.5)),
            "b2": _w((lambda *s: _rng.normal(s) * 0.05)(S) * 0.02),
        }
    _B_in = _B_setup()

    return {
        "A_x": _A_in["x"],
        "A_wqkv": _A_in["wqkv"],
        "A_wo": _A_in["wo"],
        "B_x": _B_in["x"],
        "B_w1": _B_in["w1"],
        "B_b1": _B_in["b1"],
        "B_w2": _B_in["w2"],
        "B_b2": _B_in["b2"],
    }

def reference(A_x, A_wqkv, A_wo, B_x, B_w1, B_b1, B_w2, B_b2):
    def _A_ref(x, wqkv, wo):
        B, S, D = x.shape
        H = 32; Dh = D // H
        W, dil = 8, 2
        qkv = (lambda x, *d: x.transpose(*d))((x @ wqkv).reshape(B, S, 3, H, Dh), 2, 0, 3, 1, 4)
        q, k, v = qkv[0], qkv[1], qkv[2]
        scale = Dh ** -0.5
        pos = jnp.arange(S)
        off = jnp.arange(W) * dil
        idx = pos[:, None] - off[None, :]
        mask = idx >= 0
        idx_c = jnp.where(mask, idx, 0).reshape(-1)
        kg = k[:, :, idx_c, :].reshape(B, H, S, W, Dh)
        vg = v[:, :, idx_c, :].reshape(B, H, S, W, Dh)
        logits = jnp.einsum("bhsd,bhswd->bhsw", q, kg) * scale
        logits = jnp.where(mask[None, None, :, :], logits, -1e9)
        attn = _softmax(logits, axis=-1)
        o = jnp.einsum("bhsw,bhswd->bhsd", attn, vg)
        return (lambda x, *d: x.transpose(*d))(o, 0, 2, 1, 3).reshape(B, S, D) @ wo

    def _B_ref(x, w1, b1, w2, b2):
        B, S, D = x.shape
        h = _layernorm(x, axis=-1)
        u = jnp.einsum("bsd,sf->bdf", h, w1) + b1
        u = _gelu(u)
        y = jnp.einsum("bdf,fs->bds", u, w2) + b2
        return (lambda x, *d: x.transpose(*d))(y, 0, 2, 1)

    x = A_x
    x = x + _A_ref(_layernorm(x, axis=-1), A_wqkv, A_wo)
    x = x + _B_ref(_layernorm(x, axis=-1), B_w1, B_b1, B_w2, B_b2)
    x = x + _A_ref(_layernorm(x, axis=-1), A_wqkv, A_wo)
    x = x + _B_ref(_layernorm(x, axis=-1), B_w1, B_b1, B_w2, B_b2)
    return x
```

```python
import math

import jax
import jax.numpy as jnp
from jax import lax
import jax.experimental.pallas as pl
import jax.experimental.pallas.tpu as pltpu

S, D, F = 2048, 1024, 3584
H, DH, W, DIL = 32, 32, 8, 2
HALO = 16
T = 256
NC = S // T
FC = 512
NF = F // FC
NT = D // 128
EPS = 1e-5
F32, BF16 = jnp.float32, jnp.bfloat16


def _ln(x):
    m = jnp.mean(x, axis=-1, keepdims=True)
    c = x - m
    v = jnp.mean(c * c, axis=-1, keepdims=True)
    return c * lax.rsqrt(v + EPS)


def _kernel(x_hbm, wqkv_hbm, wo_hbm, w1_hbm, b1_ref, w2_hbm, b2_ref, out_hbm,
            xin, wqkv_raw, wo_raw, w1, w2, wqkvT, wo, tmp, x, hT, g, q_s, k_s, v_s, o_s, obuf,
            sems):
    cp_x = pltpu.make_async_copy(x_hbm, xin, sems.at[0])
    cp_qkv = pltpu.make_async_copy(wqkv_hbm, wqkv_raw, sems.at[1])
    cp_wo = pltpu.make_async_copy(wo_hbm, wo_raw, sems.at[2])
    cp_w1 = [pltpu.make_async_copy(w1_hbm.at[:, pl.ds(f * FC, FC)], w1.at[f], sems.at[3]) for f in range(NF)]
    cp_w2 = [pltpu.make_async_copy(w2_hbm.at[:, pl.ds(c * T, T)], w2.at[c], sems.at[4]) for c in range(NC)]
    cp_qkv.start()
    cp_x.start()
    cp_wo.start()
    for c in cp_w1 + cp_w2:
        c.start()

    cp_qkv.wait()
    with jax.named_scope("prep"):
        for t in range(3):
            def prep_k(kt, _):
                r0 = pl.multiple_of(kt * 128, 128)
                tmp[...] = wqkv_raw[pl.ds(r0, 128), t * D:(t + 1) * D].astype(F32).T
                for d in range(DH):
                    wqkvT[kt, pl.ds(t * D + d * H, H), :] = tmp[pl.ds(d, H, stride=DH), :].astype(BF16)
            lax.fori_loop(0, NT, prep_k, None)
        cp_wo.wait()
        for nt in range(NT):
            tmp[...] = wo_raw[:, nt * 128:(nt + 1) * 128].astype(F32)
            for d in range(DH):
                wo[pl.ds(d * H, H), nt * 128:(nt + 1) * 128] = tmp[pl.ds(d, H, stride=DH), :].astype(BF16)
        cp_x.wait()
    k_s[:, 0:HALO, :] = jnp.zeros((NT, HALO, 128), F32)

    def s_load(c):
        r0 = pl.multiple_of(c * T, T)
        x[pl.ds(r0, T), :] = xin[pl.ds(r0, T), :].astype(F32)

    def s_mix2(c):
        r0 = pl.multiple_of(c * T, T)
        y = jnp.dot(g[...], w2[c], preferred_element_type=F32) + b2_ref[c].astype(F32)
        x[pl.ds(r0, T), :] += y.T

    def s_qkv(c):
        r0 = pl.multiple_of(c * T, T)
        h = _ln(x[pl.ds(r0, T), :]).astype(BF16)
        r = None
        for kt in range(NT):
            p = lax.dot_general(h[:, kt * 128:(kt + 1) * 128], wqkvT[kt], (((1,), (1,)), ((), ())),
                                preferred_element_type=F32)
            r = p if r is None else r + p
        for t in range(NT):
            q_s[t] = r[:, t * 128:(t + 1) * 128] * (DH ** -0.5)
            k_s[t, pl.ds(HALO + r0, T), :] = r[:, D + t * 128:D + (t + 1) * 128]
            v_s[t, pl.ds(HALO + r0, T), :] = r[:, 2 * D + t * 128:2 * D + (t + 1) * 128]

        @pl.when(c == 0)
        def _():
            for t in range(NT):
                v_s[t, 0:HALO, :] = jnp.broadcast_to(v_s[t, HALO:HALO + 1, :], (HALO, 128))

    def s_attn(c):
        def body(i, _):
            l0 = pl.multiple_of(i * 16, 16)
            r0 = pl.multiple_of(c * T + l0, 16)
            pos = r0 + lax.broadcasted_iota(jnp.int32, (16, 128), 0)
            q = [q_s[t, pl.ds(l0, 16), :] for t in range(NT)]
            lg = []
            for w in range(W):
                a = None
                for t in range(NT):
                    p = q[t] * k_s[t, pl.ds(r0 + HALO - DIL * w, 16), :]
                    a = p if a is None else a + p
                a = a + pltpu.roll(a, 64, 1)
                a = a + pltpu.roll(a, 32, 1)
                lg.append(jnp.where(pos >= DIL * w, a, -1e9))
            m = lg[0]
            for w in range(1, W):
                m = jnp.maximum(m, lg[w])
            e = [jnp.exp(a - m) for a in lg]
            den = e[0]
            for w in range(1, W):
                den = den + e[w]
            inv = 1.0 / den
            p = [a * inv for a in e]
            for t in range(NT):
                a = None
                for w in range(W):
                    z = p[w] * v_s[t, pl.ds(r0 + HALO - DIL * w, 16), :]
                    a = z if a is None else a + z
                o_s[pl.ds(l0, 16), t * 128:(t + 1) * 128] = a.astype(BF16)
        lax.fori_loop(0, T // 16, body, None)

    def s_wo(c):
        r0 = pl.multiple_of(c * T, T)
        xn = x[pl.ds(r0, T), :] + jnp.dot(o_s[...], wo[...], preferred_element_type=F32)
        x[pl.ds(r0, T), :] = xn
        h = _ln(_ln(xn))
        hT[c] = h.T.astype(BF16)

    def mix1():
        def body(f, _):
            u = b1_ref[f].astype(F32)
            for c in range(NC):
                u = u + jnp.dot(hT[c], w1[f, c * T:(c + 1) * T, :], preferred_element_type=F32)
            f0 = pl.multiple_of(f * FC, FC)
            g[:, pl.ds(f0, FC)] = jax.nn.gelu(u, approximate=True).astype(BF16)
        lax.fori_loop(0, NF, body, None)

    def layer(it, _):
        def body(c, _):
            @pl.when(it == 0)
            def _():
                s_load(c)

            @pl.when(it == 1)
            def _():
                with jax.named_scope("mix2"):
                    s_mix2(c)
            with jax.named_scope("qkv"):
                s_qkv(c)
            with jax.named_scope("attn"):
                s_attn(c)
            with jax.named_scope("wo"):
                s_wo(c)
        lax.fori_loop(0, NC, body, None)

        @pl.when(it == 0)
        def _():
            for c in cp_w1 + cp_w2:
                c.wait()
        with jax.named_scope("mix1"):
            mix1()
    lax.fori_loop(0, 2, layer, None)

    def fin(c, _):
        with jax.named_scope("mix2"):
            s_mix2(c)
        r0 = pl.multiple_of(c * T, T)
        obuf[pl.ds(r0, T), :] = x[pl.ds(r0, T), :].astype(BF16)
        pltpu.make_async_copy(obuf.at[pl.ds(r0, T)], out_hbm.at[pl.ds(r0, T)], sems.at[5]).start()
    lax.fori_loop(0, NC, fin, None)
    pltpu.make_async_copy(obuf, out_hbm, sems.at[5]).wait()


@jax.jit
def pallas_interleave_layers__sliding_local_dilated__mixer_token_mlp__prompt_kernel(
    A_x: jax.Array,
    A_wqkv: jax.Array,
    A_wo: jax.Array,
    B_x: jax.Array,
    B_w1: jax.Array,
    B_b1: jax.Array,
    B_w2: jax.Array,
    B_b2: jax.Array,
):
    del B_x
    hbm = pl.BlockSpec(memory_space=pl.ANY)
    vm = pl.BlockSpec(memory_space=pltpu.VMEM)
    out = pl.pallas_call(
        _kernel,
        out_shape=jax.ShapeDtypeStruct((S, D), A_x.dtype),
        in_specs=[hbm, hbm, hbm, hbm, vm, hbm, vm],
        out_specs=hbm,
        scratch_shapes=[
            pltpu.VMEM((S, D), BF16),
            pltpu.VMEM((D, 3 * D), BF16),
            pltpu.VMEM((D, D), BF16),
            pltpu.VMEM((NF, S, FC), BF16),
            pltpu.VMEM((NC, F, T), BF16),
            pltpu.VMEM((NT, 3 * D, 128), BF16),
            pltpu.VMEM((D, D), BF16),
            pltpu.VMEM((D, 128), F32),
            pltpu.VMEM((S, D), F32),
            pltpu.VMEM((NC, D, T), BF16),
            pltpu.VMEM((D, F), BF16),
            pltpu.VMEM((NT, T, 128), F32),
            pltpu.VMEM((NT, S + HALO, 128), F32),
            pltpu.VMEM((NT, S + HALO, 128), F32),
            pltpu.VMEM((T, D), BF16),
            pltpu.VMEM((S, D), BF16),
            pltpu.SemaphoreType.DMA((6,)),
        ],
        compiler_params=pltpu.CompilerParams(vmem_limit_bytes=120 * 1024 * 1024),
    )(A_x.reshape(S, D), A_wqkv, A_wo, B_w1, B_b1.reshape(NF, 1, FC), B_w2, B_b2.reshape(NC, 1, T))
    return out.reshape(1, S, D)
```

```python
import math

import jax
import jax.numpy as jnp
from jax import lax
import jax.experimental.pallas as pl
import jax.experimental.pallas.tpu as pltpu

S, D, F = 2048, 1024, 3584
H, DH, W, DIL = 32, 32, 8, 2
HALO = 16
T = 256
NC = S // T
FC = 512
NF = F // FC
NT = D // 128
NI = 1
NW = 3 * D // NI
NO = D // NI
RS = T // NI
R = 16
LR = 32
MN = 256
EPS = 1e-5
F32, BF16 = jnp.float32, jnp.bfloat16


def _ln(x):
    m = jnp.mean(x, axis=-1, keepdims=True)
    c = x - m
    v = jnp.mean(c * c, axis=-1, keepdims=True)
    return c * lax.rsqrt(v + EPS)


def _kernel(x_hbm, wqkv_hbm, wo_hbm, w1_hbm, b1_ref, w2_hbm, b2_ref, out_hbm,
            xin, wqkv_raw, wo_raw, w1, w2, wqkvT, wo, tmp, x, hT, g, qkv, h_s, h2_s, o_s, obuf,
            sems):
    cp_x = pltpu.make_async_copy(x_hbm, xin, sems.at[0])
    cp_qkv = pltpu.make_async_copy(wqkv_hbm, wqkv_raw, sems.at[1])
    cp_wo = pltpu.make_async_copy(wo_hbm, wo_raw, sems.at[2])
    cp_w1 = [pltpu.make_async_copy(w1_hbm.at[:, pl.ds(f * FC, FC)], w1.at[f], sems.at[3]) for f in range(NF)]
    cp_w2 = [pltpu.make_async_copy(w2_hbm.at[:, pl.ds(c * T, T)], w2.at[c], sems.at[4]) for c in range(NC)]
    cp_qkv.start()
    cp_x.start()
    cp_wo.start()
    for c in cp_w1 + cp_w2:
        c.start()

    cp_qkv.wait()
    with jax.named_scope("prep"):
        for t in range(3):
            def prep_k(kt, _):
                r0 = pl.multiple_of(kt * 128, 128)
                tmp[...] = wqkv_raw[pl.ds(r0, 128), t * D:(t + 1) * D].astype(F32).T
                for d in range(DH):
                    wqkvT[pl.ds(t * D + d * H, H), pl.ds(r0, 128)] = tmp[pl.ds(d, H, stride=DH), :].astype(BF16)
            lax.fori_loop(0, NT, prep_k, None)
        cp_wo.wait()
        for nt in range(NT):
            tmp[...] = wo_raw[:, nt * 128:(nt + 1) * 128].astype(F32)
            for d in range(DH):
                wo[pl.ds(d * H, H), nt * 128:(nt + 1) * 128] = tmp[pl.ds(d, H, stride=DH), :].astype(BF16)
        cp_x.wait()
    qkv[NT:2 * NT, 0:HALO, :] = jnp.zeros((NT, HALO, 128), F32)
    qkv[2 * NT:, 0:HALO, :] = jnp.zeros((NT, HALO, 128), F32)

    def s_mix2(c):
        r0 = pl.multiple_of(c * T, T)
        y = jnp.dot(g[...], w2[c], preferred_element_type=F32) + b2_ref[c].astype(F32)
        x[pl.ds(r0, T), :] += y.T

    def s_load(c):
        r0 = pl.multiple_of(c * T, T)
        x[pl.ds(r0, T), :] = xin[pl.ds(r0, T), :].astype(F32)

    def p_ln(c, j):
        r0 = pl.multiple_of(c * T, T)
        h_s[c % 2, j:j + LR, :] = _ln(x[pl.ds(r0 + j, LR), :]).astype(BF16)

    def p_ln2(c, j):
        r0 = pl.multiple_of(c * T, T)
        h2_s[j:j + LR, :] = _ln(_ln(x[pl.ds(r0 + j, LR), :])).astype(BF16)
        if (j + LR) % 128 == 0:
            hT[c, :, j + LR - 128:j + LR] = h2_s[j + LR - 128:j + LR, :].T

    def p_qkv(c, i, j):
        r0 = pl.multiple_of(c * T + HALO, HALO)
        n0 = pl.multiple_of(i * NW + j * MN, MN)
        r = lax.dot_general(h_s[c % 2], wqkvT[pl.ds(n0, MN), :], (((1,), (1,)), ((), ())),
                            preferred_element_type=F32)
        for t in range(MN // 128):
            qkv[i * (NW // 128) + j * (MN // 128) + t, pl.ds(r0, T), :] = r[:, t * 128:(t + 1) * 128]

    def p_wo(c, i, j):
        r0 = pl.multiple_of(c * T, T)
        n0 = pl.multiple_of(i * NO + j * MN, MN)
        x[pl.ds(r0, T), pl.ds(n0, MN)] += jnp.dot(o_s[c % 2], wo[:, pl.ds(n0, MN)], preferred_element_type=F32)

    def p_attn(c, i, j):
        if True:
            l0 = pl.multiple_of(i * RS + j * R, R)
            r0 = pl.multiple_of(c * T + l0 + HALO, HALO)
            pos = c * T + l0 + lax.broadcasted_iota(jnp.int32, (R, 128), 0)
            q = [qkv[t, pl.ds(r0, R), :] for t in range(NT)]
            lg = []
            for w in range(W):
                a = None
                for t in range(NT):
                    p = q[t] * qkv[NT + t, pl.ds(r0 - DIL * w, R), :]
                    a = p if a is None else a + p
                a = a + pltpu.roll(a, 64, 1)
                a = (a + pltpu.roll(a, 32, 1)) * (DH ** -0.5)
                lg.append(jnp.where(pos >= DIL * w, a, -1e9) if w else a)
            m = lg[0]
            for w in range(1, W):
                m = jnp.maximum(m, lg[w])
            e = [jnp.exp(a - m) for a in lg]
            den = e[0]
            for w in range(1, W):
                den = den + e[w]
            inv = 1.0 / den
            p = [a * inv for a in e]
            for t in range(NT):
                a = None
                for w in range(W):
                    z = p[w] * qkv[2 * NT + t, pl.ds(r0 - DIL * w, R), :]
                    a = z if a is None else a + z
                o_s[c % 2, pl.ds(l0, R), t * 128:(t + 1) * 128] = a.astype(BF16)

    def step(it, c, ln, qk, at, wo_, ln2, mix):
        if mix:
            with jax.named_scope("pre"):
                pl.when(it == 1)(lambda: s_mix2(c + 3))

        def body(i, _):
            na = RS // R
            work = [(p_qkv, c + 1, j) for j in range(NW // MN)] * qk + [(p_wo, c - 1, j) for j in range(NO // MN)] * wo_
            for j in range(na):
                for fn, cc, jj in work[j * len(work) // na:(j + 1) * len(work) // na]:
                    fn(cc, i, jj)
                if at:
                    p_attn(c, i, j)
                if (j * R) % LR == 0:
                    if ln:
                        p_ln(c + 2, j * R)
                    if ln2:
                        p_ln2(c - 2, j * R)
        if True:
            with jax.named_scope("y%d%d%d" % (qk, at, wo_)):
                body(0, None)

    def mix1():
        def body(f, _):
            u = b1_ref[f].astype(F32)
            for c in range(NC):
                u = u + jnp.dot(hT[c], w1[f, c * T:(c + 1) * T, :], preferred_element_type=F32)
            f0 = pl.multiple_of(f * FC, FC)
            g[:, pl.ds(f0, FC)] = jax.nn.gelu(u, approximate=True).astype(BF16)
        lax.fori_loop(0, NF, body, None)

    def layer(it, _):
        @pl.when(it == 1)
        def _():
            lax.fori_loop(0, 2, lambda c, _: s_mix2(c), None)
        step(it, -2, 1, 0, 0, 0, 0, 0)
        step(it, -1, 1, 1, 0, 0, 0, 1)
        for t in range(NT):
            qkv[2 * NT + t, 0:HALO, :] = jnp.broadcast_to(qkv[2 * NT + t, HALO:HALO + 1, :], (HALO, 128))
        step(it, 0, 1, 1, 1, 0, 0, 1)
        step(it, 1, 1, 1, 1, 1, 0, 1)
        lax.fori_loop(2, NC - 3, lambda c, _: step(it, c, 1, 1, 1, 1, 1, 1), None)
        step(it, NC - 3, 1, 1, 1, 1, 1, 0)
        step(it, NC - 2, 0, 1, 1, 1, 1, 0)
        step(it, NC - 1, 0, 0, 1, 1, 1, 0)
        step(it, NC, 0, 0, 0, 1, 1, 0)
        step(it, NC + 1, 0, 0, 0, 0, 1, 0)

        @pl.when(it == 0)
        def _():
            for c in cp_w1 + cp_w2:
                c.wait()
        with jax.named_scope("mix1"):
            mix1()
    lax.fori_loop(0, NC, lambda c, _: s_load(c), None)
    lax.fori_loop(0, 2, layer, None)

    def fin(c, _):
        with jax.named_scope("mix2"):
            s_mix2(c)
        r0 = pl.multiple_of(c * T, T)
        obuf[pl.ds(r0, T), :] = x[pl.ds(r0, T), :].astype(BF16)
        pltpu.make_async_copy(obuf.at[pl.ds(r0, T)], out_hbm.at[pl.ds(r0, T)], sems.at[5]).start()
    lax.fori_loop(0, NC, fin, None)
    pltpu.make_async_copy(obuf, out_hbm, sems.at[5]).wait()


@jax.jit
def pallas_interleave_layers__sliding_local_dilated__mixer_token_mlp__prompt_kernel(
    A_x: jax.Array,
    A_wqkv: jax.Array,
    A_wo: jax.Array,
    B_x: jax.Array,
    B_w1: jax.Array,
    B_b1: jax.Array,
    B_w2: jax.Array,
    B_b2: jax.Array,
):
    del B_x
    hbm = pl.BlockSpec(memory_space=pl.ANY)
    vm = pl.BlockSpec(memory_space=pltpu.VMEM)
    out = pl.pallas_call(
        _kernel,
        out_shape=jax.ShapeDtypeStruct((S, D), A_x.dtype),
        in_specs=[hbm, hbm, hbm, hbm, vm, hbm, vm],
        out_specs=hbm,
        scratch_shapes=[
            pltpu.VMEM((S, D), BF16),
            pltpu.VMEM((D, 3 * D), BF16),
            pltpu.VMEM((D, D), BF16),
            pltpu.VMEM((NF, S, FC), BF16),
            pltpu.VMEM((NC, F, T), BF16),
            pltpu.VMEM((3 * D, D), BF16),
            pltpu.VMEM((D, D), BF16),
            pltpu.VMEM((D, 128), F32),
            pltpu.VMEM((S, D), F32),
            pltpu.VMEM((NC, D, T), BF16),
            pltpu.VMEM((D, F), BF16),
            pltpu.VMEM((3 * NT, S + HALO, 128), F32),
            pltpu.VMEM((2, T, D), BF16),
            pltpu.VMEM((T, D), BF16),
            pltpu.VMEM((2, T, D), BF16),
            pltpu.VMEM((S, D), BF16),
            pltpu.SemaphoreType.DMA((6,)),
        ],
        compiler_params=pltpu.CompilerParams(vmem_limit_bytes=120 * 1024 * 1024),
    )(A_x.reshape(S, D), A_wqkv, A_wo, B_w1, B_b1.reshape(NF, 1, FC), B_w2, B_b2.reshape(NC, 1, T))
    return out.reshape(1, S, D)
```

```python
import math

import jax
import jax.numpy as jnp
from jax import lax
import jax.experimental.pallas as pl
import jax.experimental.pallas.tpu as pltpu

S, D, F = 2048, 1024, 3584
H, DH, W, DIL = 32, 32, 8, 2
HALO = 16
T = 256
NC = S // T
FC = 512
NF = F // FC
NT = D // 128
NI = 1
NW = 3 * D // NI
NO = D // NI
RS = T // NI
R = 16
LR = 32
MN = 256
LO = 8
PS = 33
EPS = 1e-5
F32, BF16 = jnp.float32, jnp.bfloat16


def _ln(x):
    m = jnp.mean(x, axis=-1, keepdims=True)
    c = x - m
    v = jnp.mean(c * c, axis=-1, keepdims=True)
    return c * lax.rsqrt(v + EPS)


def _kernel(x_hbm, wqkv_hbm, wo_hbm, w1_hbm, b1_ref, w2_hbm, b2_ref, out_hbm,
            xin, wqkv_raw, wo_raw, w1, w2, wqkvT, wo, tmp, x, hT, g, qkv, h_s, h2_s, o_s, obuf,
            sems):
    cp_x = pltpu.make_async_copy(x_hbm, xin, sems.at[0])
    cp_qkv = [pltpu.make_async_copy(wqkv_hbm.at[:, pl.ds(t * D, D)], wqkv_raw.at[t], sems.at[6 + t]) for t in range(3)]
    cp_wo = pltpu.make_async_copy(wo_hbm, wo_raw, sems.at[2])
    cp_w1 = [pltpu.make_async_copy(w1_hbm.at[:, pl.ds(f * FC, FC)], w1.at[f], sems.at[3]) for f in range(NF)]
    cp_w2 = [pltpu.make_async_copy(w2_hbm.at[:, pl.ds(c * T, T)], w2.at[c], sems.at[4]) for c in range(NC)]
    cp_qkv[0].start(priority=0)
    cp_qkv[1].start()
    cp_qkv[2].start()
    cp_wo.start()
    cp_x.start()

    def put(a):
        for h in range(H):
            tmp[h * PS:h * PS + DH, :] = a[h * DH:(h + 1) * DH]

    with jax.named_scope("prep"):
        for t in range(3):
            cp_qkv[t].wait()

            def prep_k(kt, _):
                r0 = pl.multiple_of(kt * 128, 128)
                put(wqkv_raw[t, pl.ds(r0, 128), :].astype(F32).T)
                for d in range(DH):
                    wqkvT[pl.ds(t * D + d * H, H), pl.ds(r0, 128)] = tmp[pl.ds(d, H, stride=PS), :].astype(BF16)
            lax.fori_loop(0, NT, prep_k, None)
        cp_wo.wait()
        for c in cp_w1 + cp_w2:
            c.start()
        for nt in range(NT):
            put(wo_raw[:, nt * 128:(nt + 1) * 128].astype(F32))
            for d in range(DH):
                wo[pl.ds(d * H, H), nt * 128:(nt + 1) * 128] = tmp[pl.ds(d, H, stride=PS), :].astype(BF16)
        cp_x.wait()
    qkv[NT:2 * NT, 0:HALO, :] = jnp.zeros((NT, HALO, 128), F32)
    qkv[2 * NT:, 0:HALO, :] = jnp.zeros((NT, HALO, 128), F32)

    def s_mix2(c):
        r0 = pl.multiple_of(c * T, T)
        y = jnp.dot(g[...], w2[c], preferred_element_type=F32) + b2_ref[c].astype(F32)
        x[pl.ds(r0, T), :] += y.T

    def s_load(c):
        r0 = pl.multiple_of(c * T, T)
        x[pl.ds(r0, T), :] = xin[pl.ds(r0, T), :].astype(F32)

    def p_ln(c, j):
        r0 = pl.multiple_of(c * T, T)
        h_s[c % 2, j:j + LR, :] = _ln(x[pl.ds(r0 + j, LR), :]).astype(BF16)

    def p_ln2(c, j):
        r0 = pl.multiple_of(c * T, T)
        h2_s[j:j + LR, :] = _ln(_ln(x[pl.ds(r0 + j, LR), :])).astype(BF16)
        if (j + LR) % 128 == 0:
            hT[c, :, j + LR - 128:j + LR] = h2_s[j + LR - 128:j + LR, :].T

    def p_qkv(c, i, j):
        r0 = pl.multiple_of(c * T + HALO, HALO)
        n0 = pl.multiple_of(i * NW + j * MN, MN)
        r = lax.dot_general(h_s[c % 2], wqkvT[pl.ds(n0, MN), :], (((1,), (1,)), ((), ())),
                            preferred_element_type=F32)
        for t in range(MN // 128):
            qkv[i * (NW // 128) + j * (MN // 128) + t, pl.ds(r0, T), :] = r[:, t * 128:(t + 1) * 128]

    def p_wo(c, i, j):
        r0 = pl.multiple_of(c * T, T)
        n0 = pl.multiple_of(i * NO + j * MN, MN)
        x[pl.ds(r0, T), pl.ds(n0, MN)] += jnp.dot(o_s[c % 2], wo[:, pl.ds(n0, MN)], preferred_element_type=F32)

    def p_attn(c, i, j):
        if True:
            l0 = pl.multiple_of(i * RS + j * R, R)
            r0 = pl.multiple_of(c * T + l0 + HALO, HALO)
            pos = c * T + l0 + lax.broadcasted_iota(jnp.int32, (R, 128), 0)
            q = [qkv[t, pl.ds(r0, R), :] for t in range(NT)]
            lg = []
            for w in range(W):
                a = None
                for t in range(NT):
                    p = q[t] * qkv[NT + t, pl.ds(r0 - DIL * w, R), :]
                    a = p if a is None else a + p
                a = a + pltpu.roll(a, 64, 1)
                a = (a + pltpu.roll(a, 32, 1)) * (DH ** -0.5)
                lg.append(jnp.where(pos >= DIL * w, a, -1e9) if w else a)
            m = lg[0]
            for w in range(1, W):
                m = jnp.maximum(m, lg[w])
            e = [jnp.exp(a - m) for a in lg]
            den = e[0]
            for w in range(1, W):
                den = den + e[w]
            inv = 1.0 / den
            p = [a * inv for a in e]
            for t in range(NT):
                a = None
                for w in range(W):
                    z = p[w] * qkv[2 * NT + t, pl.ds(r0 - DIL * w, R), :]
                    a = z if a is None else a + z
                o_s[c % 2, pl.ds(l0, R), t * 128:(t + 1) * 128] = a.astype(BF16)

    def step(it, c, ln, qk, at, wo_, ln2, mix):
        def body(i, _):
            na = RS // R
            work = [(p_qkv, c + 1, j) for j in range(NW // MN)] * qk + [(p_wo, c - 1, j) for j in range(NO // MN)] * wo_
            for j in range(na):
                for fn, cc, jj in work[j * len(work) // na:(j + 1) * len(work) // na]:
                    fn(cc, i, jj)
                if at:
                    p_attn(c, i, j)
                if ln2 and j < T // LR:
                    p_ln2(c - 2, j * LR)
                if ln and LO <= j < LO + T // LR:
                    p_ln(c + 2, (j - LO) * LR)
        if True:
            with jax.named_scope("y%d%d%d" % (qk, at, wo_)):
                body(0, None)

    def mix1():
        def body(f, _):
            u = b1_ref[f].astype(F32)
            for c in range(NC):
                u = u + jnp.dot(hT[c], w1[f, c * T:(c + 1) * T, :], preferred_element_type=F32)
            f0 = pl.multiple_of(f * FC, FC)
            g[:, pl.ds(f0, FC)] = jax.nn.gelu(u, approximate=True).astype(BF16)
        lax.fori_loop(0, NF, body, None)

    def layer(it, _):
        step(it, -2, 1, 0, 0, 0, 0, 0)
        step(it, -1, 1, 1, 0, 0, 0, 1)
        for t in range(NT):
            qkv[2 * NT + t, 0:HALO, :] = jnp.broadcast_to(qkv[2 * NT + t, HALO:HALO + 1, :], (HALO, 128))
        step(it, 0, 1, 1, 1, 0, 0, 1)
        step(it, 1, 1, 1, 1, 1, 0, 1)
        lax.fori_loop(2, NC - 2, lambda c, _: step(it, c, 1, 1, 1, 1, 1, 1), None)
        step(it, NC - 2, 0, 1, 1, 1, 1, 0)
        step(it, NC - 1, 0, 0, 1, 1, 1, 0)
        step(it, NC, 0, 0, 0, 1, 1, 0)
        step(it, NC + 1, 0, 0, 0, 0, 1, 0)

        @pl.when(it == 0)
        def _():
            for c in cp_w1 + cp_w2:
                c.wait()
        with jax.named_scope("mix1"):
            mix1()

        def fin(c, _):
            with jax.named_scope("mix2"):
                s_mix2(c)

            @pl.when(it == 1)
            def _():
                r0 = pl.multiple_of(c * T, T)
                obuf[pl.ds(r0, T), :] = x[pl.ds(r0, T), :].astype(BF16)
                pltpu.make_async_copy(obuf.at[pl.ds(r0, T)], out_hbm.at[pl.ds(r0, T)], sems.at[5]).start()
        lax.fori_loop(0, NC, fin, None)
    lax.fori_loop(0, NC, lambda c, _: s_load(c), None)
    lax.fori_loop(0, 2, layer, None)

    pltpu.make_async_copy(obuf, out_hbm, sems.at[5]).wait()


@jax.jit
def pallas_interleave_layers__sliding_local_dilated__mixer_token_mlp__prompt_kernel(
    A_x: jax.Array,
    A_wqkv: jax.Array,
    A_wo: jax.Array,
    B_x: jax.Array,
    B_w1: jax.Array,
    B_b1: jax.Array,
    B_w2: jax.Array,
    B_b2: jax.Array,
):
    del B_x
    hbm = pl.BlockSpec(memory_space=pl.ANY)
    vm = pl.BlockSpec(memory_space=pltpu.VMEM)
    out = pl.pallas_call(
        _kernel,
        out_shape=jax.ShapeDtypeStruct((S, D), A_x.dtype),
        in_specs=[hbm, hbm, hbm, hbm, vm, hbm, vm],
        out_specs=hbm,
        scratch_shapes=[
            pltpu.VMEM((S, D), BF16),
            pltpu.VMEM((3, D, D), BF16),
            pltpu.VMEM((D, D), BF16),
            pltpu.VMEM((NF, S, FC), BF16),
            pltpu.VMEM((NC, F, T), BF16),
            pltpu.VMEM((3 * D, D), BF16),
            pltpu.VMEM((D, D), BF16),
            pltpu.VMEM((H * PS, 128), F32),
            pltpu.VMEM((S, D), F32),
            pltpu.VMEM((NC, D, T), BF16),
            pltpu.VMEM((D, F), BF16),
            pltpu.VMEM((3 * NT, S + HALO, 128), F32),
            pltpu.VMEM((2, T, D), BF16),
            pltpu.VMEM((T, D), BF16),
            pltpu.VMEM((2, T, D), BF16),
            pltpu.VMEM((S, D), BF16),
            pltpu.SemaphoreType.DMA((9,)),
        ],
        compiler_params=pltpu.CompilerParams(vmem_limit_bytes=120 * 1024 * 1024),
    )(A_x.reshape(S, D), A_wqkv, A_wo, B_w1, B_b1.reshape(NF, 1, FC), B_w2, B_b2.reshape(NC, 1, T))
    return out.reshape(1, S, D)
```

```python
import jax
import jax.numpy as jnp
from jax import lax
import jax.experimental.pallas as pl
import jax.experimental.pallas.tpu as pltpu

S, D, F = 2048, 1024, 3584
H, DH, W, DIL = 32, 32, 8, 2
HALO = 16
T = 256
NC = S // T
NT = D // 128
MN = 256
R = 16
LR = 32
LO = 8
FC = 512
NF = F // FC
T2 = 512
N2 = S // T2
DM, FH, TH = D // 2, FC // 2, T2 // 2
PS = DH + 1
KP = 4
EPS = 1e-5
F32, BF16, U32 = jnp.float32, jnp.bfloat16, jnp.uint32


def _ln(x):
    m = jnp.mean(x, axis=-1, keepdims=True)
    c = x - m
    v = jnp.mean(c * c, axis=-1, keepdims=True)
    return c * lax.rsqrt(v + EPS)


def _pack(a):
    return pltpu.bitcast(a.astype(BF16), U32)


def _unpack(a):
    return pltpu.bitcast(a, BF16)


def _lhs7(a11, a12, a21, a22):
    return (a11 + a22, a21 + a22, a11, a22, a11 + a12, a21 - a11, a12 - a22)


def _rhs(i, b):
    if i in (1, 4):
        return b(0, 0) if i == 1 else b(1, 1)
    p, q, add = {0: ((0, 0), (1, 1), True), 2: ((0, 1), (1, 1), False), 3: ((1, 0), (0, 0), False),
                 5: ((0, 0), (0, 1), True), 6: ((1, 0), (1, 1), True)}[i]
    p, q = b(*p).astype(F32), b(*q).astype(F32)
    return (p + q if add else p - q).astype(BF16)


def _out4(m):
    return (m[0] + m[3] - m[4] + m[6], m[2] + m[4], m[1] + m[3], m[0] - m[1] + m[2] + m[5])


def _weave(*streams):
    items = [((j + 0.5 * (s > 0)) / len(st), s, j) for s, st in enumerate(streams) for j in range(len(st))]
    for _, s, j in sorted(items):
        streams[s][j]()


def _at(c, n, off=0):
    return c * n + off if isinstance(c, int) else pl.multiple_of(c * n + off, 16)


def _kernel(x_hbm, wqkv_hbm, wo_hbm, w1_hbm, b1_ref, w2_hbm, b2_ref, out_hbm,
            xio, raw, w1, w2, wqT, wkT, wvT, wo, tmp, x, hS, gS, mb, q_s, k_s, v_s, h_s, h2_s, o_s, sems):
    dma = pltpu.make_async_copy
    kp = D // KP
    cp_x0 = dma(x_hbm.at[0:2 * T], xio.at[0:2 * T], sems.at[0])
    cp_x1 = dma(x_hbm.at[2 * T:S], xio.at[2 * T:S], sems.at[1])
    cp_k = dma(wqkv_hbm.at[:, D:2 * D], raw.at[1], sems.at[2])
    cp_v = dma(wqkv_hbm.at[:, 2 * D:3 * D], raw.at[2], sems.at[3])
    cp_o = dma(wo_hbm, raw.at[3], sems.at[4])
    cp_w = [dma(w1_hbm.at[:, f * FC:(f + 1) * FC], w1.at[f], sems.at[5]) for f in range(NF)]
    cp_w += [dma(w2_hbm.at[:, c * T2:(c + 1) * T2], w2.at[c], sems.at[6]) for c in range(N2)]
    cp_q = [dma(wqkv_hbm.at[p * kp:(p + 1) * kp, 0:D], raw.at[0, p * kp:(p + 1) * kp], sems.at[8 + p])
            for p in range(KP)]

    def prep(t, kt):
        c0 = _at(kt, 128)
        a = raw[t, pl.ds(c0, 128), :].astype(F32).T if t < 3 else raw[t, :, pl.ds(c0, 128)].astype(F32)
        for h in range(H):
            tmp[kt % 2, h * PS:h * PS + DH, :] = a[h * DH:(h + 1) * DH]
        dst = (wqT, wkT, wvT, wo)[t]
        for d in range(DH):
            dst[d * H // 2:(d + 1) * H // 2, pl.ds(c0, 128)] = _pack(tmp[kt % 2, pl.ds(d, H, stride=PS), :])

    def p_ln(it, c, j):
        rows = pl.ds(_at(c, T, j), LR)
        h_s[c % 2, j // 2:(j + LR) // 2, :] = _pack(_ln(x[rows, :] if it else xio[rows, :].astype(F32)))

    def p_qkv(c, t, j):
        w = (wqT, wkT, wvT)[t][j * MN // 2:(j + 1) * MN // 2, :]
        r = lax.dot_general(_unpack(h_s[c % 2]), _unpack(w), (((1,), (1,)), ((), ())), preferred_element_type=F32)
        for u in range(MN // 128):
            val, n = r[:, u * 128:(u + 1) * 128], j * (MN // 128) + u
            if t == 0:
                q_s[c % 2, n] = val
            else:
                (k_s, v_s)[t - 1][n, pl.ds(_at(c, T, HALO), T), :] = val

    def p_attn(c, j):
        r0 = _at(c, T, j * R + HALO)
        q = [q_s[c % 2, t, j * R:(j + 1) * R, :] for t in range(NT)]
        lg = []
        for w in range(W):
            a = q[0] * k_s[0, pl.ds(r0 - DIL * w, R), :]
            for t in range(1, NT):
                a = a + q[t] * k_s[t, pl.ds(r0 - DIL * w, R), :]
            a = a + pltpu.roll(a, 64, 1)
            a = (a + pltpu.roll(a, 32, 1)) * (DH ** -0.5)
            if isinstance(c, int) and c * T + j * R < DIL * w:
                a = jnp.where(c * T + j * R + lax.broadcasted_iota(jnp.int32, (R, 128), 0) >= DIL * w, a, -1e9)
            lg.append(a)
        m = lg[0]
        for w in range(1, W):
            m = jnp.maximum(m, lg[w])
        e = [jnp.exp(a - m) for a in lg]
        den = e[0]
        for w in range(1, W):
            den = den + e[w]
        inv = 1.0 / den
        p = [a * inv for a in e]
        for t in range(NT):
            a = p[0] * v_s[t, pl.ds(r0, R), :]
            for w in range(1, W):
                a = a + p[w] * v_s[t, pl.ds(r0 - DIL * w, R), :]
            o_s[c % 2, j * R // 2:(j + 1) * R // 2, t * 128:(t + 1) * 128] = _pack(a)

    def p_wo(it, c, j):
        rows, cols = pl.ds(_at(c, T), T), slice(j * MN, (j + 1) * MN)
        r = jnp.dot(_unpack(o_s[c % 2]), _unpack(wo[:, cols]), preferred_element_type=F32)
        x[rows, cols] = (x[rows, cols] if it else xio[rows, cols].astype(F32)) + r

    def p_ln2(c, j):
        h2_s[j:j + LR, :] = _ln(_ln(x[pl.ds(_at(c, T, j), LR), :]))

    def p_hT(c, j):
        a = [h2_s[k * 128:(k + 1) * 128, r * DM + j * 128:r * DM + (j + 1) * 128].T for r in (0, 1) for k in (0, 1)]
        for i, v in enumerate(_lhs7(*a)):
            hS[i, j * 64:(j + 1) * 64, pl.ds(_at(c, 128), 128)] = _pack(v)

    def m1(f, i, c0=0, c1=NC):
        def b(k, n):
            return jnp.concatenate(
                [w1[f, c * T + k * 128:c * T + (k + 1) * 128, n * FH:(n + 1) * FH] for c in range(c0, c1)], axis=0)
        r = jnp.dot(_unpack(hS[i, :, c0 * 128:c1 * 128]), _rhs(i, b), preferred_element_type=F32)
        mb[f % 2, i] = r + mb[f % 2, i] if c0 else r

    def e1(f, j):
        rows = slice(j * 32, (j + 1) * 32)
        bias = b1_ref[f].astype(F32)
        u = _out4([mb[f % 2, i, rows, :] for i in range(7)])
        g = [jax.nn.gelu(v + bias[:, (n % 2) * FH:(n % 2 + 1) * FH], approximate=True) for n, v in enumerate(u)]
        for i, v in enumerate(_lhs7(*g)):
            gS[i, j * 16:(j + 1) * 16, pl.ds(_at(f, FH), FH)] = _pack(v)

    def m2(c, i, f0=0, f1=NF):
        def b(k, n):
            return jnp.concatenate(
                [w2[c, f * FC + k * FH:f * FC + (k + 1) * FH, n * TH:(n + 1) * TH] for f in range(f0, f1)], axis=0)
        r = jnp.dot(_unpack(gS[i, :, f0 * FH:f1 * FH]), _rhs(i, b), preferred_element_type=F32)
        mb[(c + NF) % 2, i] = r + mb[(c + NF) % 2, i] if f0 else r

    def e2(it, c, j, k):
        rows, cols = slice(j * 128, (j + 1) * 128), slice(k * 128, (k + 1) * 128)
        y = _out4([mb[(c + NF) % 2, i, rows, cols] for i in range(7)])
        for n, v in enumerate(y):
            t0 = (n % 2) * TH + k * 128
            tok, ch = pl.ds(_at(c, T2, t0), 128), slice((n // 2) * DM + j * 128, (n // 2) * DM + (j + 1) * 128)
            res = x[tok, ch] + (v + b2_ref[c, :, t0:t0 + 128].astype(F32)).T
            if it:
                xio[tok, ch] = res.astype(BF16)
            else:
                x[tok, ch] = res

    def send(c):
        rows = pl.ds(_at(c, T2), T2)
        dma(xio.at[rows], out_hbm.at[rows], sems.at[7]).start()

    def each(fn, *a, n, step=1):
        return [lambda j=j: fn(*a, j) for j in range(0, n, step)]

    def l_e2(it, c):
        return [lambda j=j, k=k: e2(it, c, j, k) for k in range(TH // 128) for j in range(DM // 128)]

    def l_m(fn, c, *rng):
        return [lambda i=i: fn(c, i, *rng) for i in range(7)]

    def step(it, c, qk=1, at=1, wo_=1, ln=1, ln2=1, mm=()):
        mx = [f for t in range(3) for f in each(p_qkv, c + 1, t, n=D // MN)] * qk
        mx += each(p_wo, it, c - 1, n=D // MN) * wo_ + list(mm)
        nm = (each(p_ln2, c - 2, n=T, step=LR) + each(p_hT, c - 2, n=DM // 128)) * ln2
        nm += each(p_ln, it, c + 2, n=T, step=LR) * ln
        with jax.named_scope("y%d%d%d" % (qk, at, wo_)):
            _weave(mx, each(p_attn, c, n=T // R) * at, nm)

    def v_halo():
        for t in range(NT):
            k_s[t, 0:HALO, :] = jnp.broadcast_to(k_s[t, HALO:HALO + 1, :], (HALO, 128))
            v_s[t, 0:HALO, :] = jnp.broadcast_to(v_s[t, HALO:HALO + 1, :], (HALO, 128))

    with jax.named_scope("start"):
        cp_x0.start()
        for cp in cp_q:
            cp.start()
        cp_k.start()
        cp_x0.wait()
        _weave(each(p_ln, 0, 0, n=T, step=LR) + each(p_ln, 0, 1, n=T, step=LR))
        for p in range(KP):
            cp_q[p].wait()
            if p == KP - 1:
                cp_v.start()
            _weave(each(prep, 0, n=NT)[p * NT // KP:(p + 1) * NT // KP])
    with jax.named_scope("start2"):
        for t, (cur, nxt) in enumerate(((cp_k, [cp_o]), (cp_v, [cp_x1]), (cp_o, cp_w))):
            cur.wait()
            for cp in nxt:
                cp.start()
            _weave(each(p_qkv, 0, t, n=D // MN), each(prep, t + 1, n=NT))
        cp_x1.wait()

    for it in range(2):
        v_halo()
        step(it, 0, wo_=0, ln2=0)
        step(it, 1, ln2=0)
        lax.fori_loop(2, NC - 2, lambda c, _, it=it: step(it, c), None)
        step(it, NC - 2, ln=0)
        if it == 0:
            for cp in cp_w:
                cp.wait()
        step(it, NC - 1, qk=0, ln=0, mm=l_m(m1, 0, 0, NC - 3))
        step(it, NC, qk=0, at=0, ln=0)
        step(it, NC + 1, qk=0, at=0, wo_=0, ln=0, mm=l_m(m1, 0, NC - 3, NC - 1))
        with jax.named_scope("mix1"):
            _weave(l_m(m1, 0, NC - 1, NC))
            lax.fori_loop(1, NF, lambda f, _: _weave(l_m(m1, f), each(e1, f - 1, n=DM // 32)), None)
        with jax.named_scope("mix2"):
            _weave(l_m(m2, 0, 0, NF - 1), each(e1, NF - 1, n=DM // 32))
            _weave(l_m(m2, 0, NF - 1, NF))

            def body(c, _, it=it):
                _weave(l_m(m2, c), l_e2(it, c - 1))
                if it:
                    send(c - 1)
            lax.fori_loop(1, N2, body, None)
        with jax.named_scope("turn"):
            if it == 0:
                _weave(each(p_ln, 1, 0, n=T, step=LR))
                _weave([f for t in range(3) for f in each(p_qkv, 0, t, n=D // MN)],
                       l_e2(0, N2 - 1) + each(p_ln, 1, 1, n=T, step=LR))
            else:
                _weave(l_e2(1, N2 - 1))
                send(N2 - 1)
    dma(xio, out_hbm, sems.at[7]).wait()


@jax.jit
def pallas_interleave_layers__sliding_local_dilated__mixer_token_mlp__prompt_kernel(
    A_x: jax.Array,
    A_wqkv: jax.Array,
    A_wo: jax.Array,
    B_x: jax.Array,
    B_w1: jax.Array,
    B_b1: jax.Array,
    B_w2: jax.Array,
    B_b2: jax.Array,
):
    del B_x
    hbm = pl.BlockSpec(memory_space=pl.ANY)
    vm = pl.BlockSpec(memory_space=pltpu.VMEM)
    out = pl.pallas_call(
        _kernel,
        out_shape=jax.ShapeDtypeStruct((S, D), A_x.dtype),
        in_specs=[hbm, hbm, hbm, hbm, vm, hbm, vm],
        out_specs=hbm,
        scratch_shapes=[
            pltpu.VMEM((S, D), BF16),
            pltpu.VMEM((4, D, D), BF16),
            pltpu.VMEM((NF, S, FC), BF16),
            pltpu.VMEM((N2, F, T2), BF16),
            pltpu.VMEM((D // 2, D), U32),
            pltpu.VMEM((D // 2, D), U32),
            pltpu.VMEM((D // 2, D), U32),
            pltpu.VMEM((D // 2, D), U32),
            pltpu.VMEM((2, H * PS, 128), F32),
            pltpu.VMEM((S, D), F32),
            pltpu.VMEM((7, DM // 2, S // 2), U32),
            pltpu.VMEM((7, DM // 2, F // 2), U32),
            pltpu.VMEM((2, 7, DM, FH), F32),
            pltpu.VMEM((2, NT, T, 128), F32),
            pltpu.VMEM((NT, S + HALO, 128), F32),
            pltpu.VMEM((NT, S + HALO, 128), F32),
            pltpu.VMEM((2, T // 2, D), U32),
            pltpu.VMEM((T, D), F32),
            pltpu.VMEM((2, T // 2, D), U32),
            pltpu.SemaphoreType.DMA((8 + KP,)),
        ],
        compiler_params=pltpu.CompilerParams(vmem_limit_bytes=126 * 1024 * 1024),
    )(A_x.reshape(S, D), A_wqkv, A_wo, B_w1, B_b1.reshape(NF, 1, FC), B_w2, B_b2.reshape(N2, 1, T2))
    return out.reshape(1, S, D)
```

```python
import jax
import jax.numpy as jnp
from jax import lax
import jax.experimental.pallas as pl
import jax.experimental.pallas.tpu as pltpu

S, D, F = 2048, 1024, 3584
H, DH, W, DIL = 32, 32, 8, 2
HALO = 16
T = 256
NC = S // T
NT = D // 128
MN = 256
R = 16
LR = 32
U2 = 1
FC = 512
NF = F // FC
T2 = 512
N2 = S // T2
DM, FH, TH = D // 2, FC // 2, T2 // 2
PS = DH + 1
KP = 4
EPS = 1e-5
F32, BF16, U32 = jnp.float32, jnp.bfloat16, jnp.uint32


def _ln(x):
    m = jnp.mean(x, axis=-1, keepdims=True)
    c = x - m
    v = jnp.mean(c * c, axis=-1, keepdims=True)
    return c * lax.rsqrt(v + EPS)


def _pack(a):
    return pltpu.bitcast(a.astype(BF16), U32)


def _unpack(a):
    return pltpu.bitcast(a, BF16)


def _lhs7(a11, a12, a21, a22):
    return (a11 + a22, a21 + a22, a11, a22, a11 + a12, a21 - a11, a12 - a22)


def _rhs(i, b):
    if i in (1, 4):
        return b(0, 0) if i == 1 else b(1, 1)
    p, q, add = {0: ((0, 0), (1, 1), True), 2: ((0, 1), (1, 1), False), 3: ((1, 0), (0, 0), False),
                 5: ((0, 0), (0, 1), True), 6: ((1, 0), (1, 1), True)}[i]
    p, q = b(*p).astype(F32), b(*q).astype(F32)
    return (p + q if add else p - q).astype(BF16)


def _out4(m):
    return (m[0] + m[3] - m[4] + m[6], m[2] + m[4], m[1] + m[3], m[0] - m[1] + m[2] + m[5])


def _weave(*streams):
    items = [((j + 0.5 * (s > 0)) / len(st), s, j) for s, st in enumerate(streams) for j in range(len(st))]
    for _, s, j in sorted(items):
        streams[s][j]()


def _loop(lo, hi, body, unroll):
    if unroll:
        for i in range(lo, hi):
            body(i, None)
    else:
        lax.fori_loop(lo, hi, body, None)


def _at(c, n, off=0):
    return c * n + off if isinstance(c, int) else pl.multiple_of(c * n + off, 16)


def _kernel(x_hbm, wqkv_hbm, wo_hbm, w1_hbm, b1_ref, w2_hbm, b2_ref, out_hbm,
            xio, raw, w1, w2, wqT, wkT, wvT, wo, tmp, x, hS, gS, mb, q_s, k_s, v_s, h_s, h2_s, o_s, sems):
    dma = pltpu.make_async_copy
    kp = D // KP
    cp_x0 = dma(x_hbm.at[0:2 * T], xio.at[0:2 * T], sems.at[0])
    cp_x1 = dma(x_hbm.at[2 * T:3 * T], xio.at[2 * T:3 * T], sems.at[1])
    cp_x2 = dma(x_hbm.at[3 * T:S], xio.at[3 * T:S], sems.at[8])
    cp_k = dma(wqkv_hbm.at[:, D:2 * D], raw.at[1], sems.at[2])
    cp_v = dma(wqkv_hbm.at[:, 2 * D:3 * D], raw.at[2], sems.at[3])
    cp_o = dma(wo_hbm, raw.at[3], sems.at[4])
    cp_w = [dma(w1_hbm.at[:, f * FC:(f + 1) * FC], w1.at[f], sems.at[5]) for f in range(NF)]
    cp_w += [dma(w2_hbm.at[:, c * T2:(c + 1) * T2], w2.at[c], sems.at[6]) for c in range(N2)]
    cp_q = [dma(wqkv_hbm.at[p * kp:(p + 1) * kp, 0:D], raw.at[0, p * kp:(p + 1) * kp], sems.at[9 + p])
            for p in range(KP)]

    def prep(t, kt):
        c0 = _at(kt, 128)
        a = raw[t, pl.ds(c0, 128), :].astype(F32).T if t < 3 else raw[t, :, pl.ds(c0, 128)].astype(F32)
        for h in range(H):
            tmp[kt % 2, h * PS:h * PS + DH, :] = a[h * DH:(h + 1) * DH]
        dst = (wqT, wkT, wvT, wo)[t]
        for d in range(DH):
            dst[d * H // 2:(d + 1) * H // 2, pl.ds(c0, 128)] = _pack(tmp[kt % 2, pl.ds(d, H, stride=PS), :])

    def p_ln(it, c, j):
        rows = pl.ds(_at(c if isinstance(c, int) else jnp.minimum(c, NC - 1), T, j), LR)
        h_s[c % 2, j // 2:(j + LR) // 2, :] = _pack(_ln(x[rows, :] if it else xio[rows, :].astype(F32)))

    def p_qkv(c, t, j):
        w = (wqT, wkT, wvT)[t][j * MN // 2:(j + 1) * MN // 2, :]
        r = lax.dot_general(_unpack(h_s[c % 2]), _unpack(w), (((1,), (1,)), ((), ())), preferred_element_type=F32)
        for u in range(MN // 128):
            val, n = r[:, u * 128:(u + 1) * 128], j * (MN // 128) + u
            if t == 0:
                q_s[c % 2, n] = val
            else:
                (k_s, v_s)[t - 1][n, pl.ds(_at(c, T, HALO), T), :] = val

    def p_attn(c, j):
        r0 = _at(c, T, j * R + HALO)
        q = [q_s[c % 2, t, j * R:(j + 1) * R, :] for t in range(NT)]
        lg = []
        for w in range(W):
            a = q[0] * k_s[0, pl.ds(r0 - DIL * w, R), :]
            for t in range(1, NT):
                a = a + q[t] * k_s[t, pl.ds(r0 - DIL * w, R), :]
            a = a + pltpu.roll(a, 64, 1)
            a = (a + pltpu.roll(a, 32, 1)) * (DH ** -0.5)
            if isinstance(c, int) and c * T + j * R < DIL * w:
                a = jnp.where(c * T + j * R + lax.broadcasted_iota(jnp.int32, (R, 128), 0) >= DIL * w, a, -1e9)
            lg.append(a)
        m = lg[0]
        for w in range(1, W):
            m = jnp.maximum(m, lg[w])
        e = [jnp.exp(a - m) for a in lg]
        den = e[0]
        for w in range(1, W):
            den = den + e[w]
        inv = 1.0 / den
        p = [a * inv for a in e]
        for t in range(NT):
            a = p[0] * v_s[t, pl.ds(r0, R), :]
            for w in range(1, W):
                a = a + p[w] * v_s[t, pl.ds(r0 - DIL * w, R), :]
            o_s[c % 2, j * R // 2:(j + 1) * R // 2, t * 128:(t + 1) * 128] = _pack(a)

    def p_wo(it, c, j):
        rows, cols = pl.ds(_at(c, T), T), slice(j * MN, (j + 1) * MN)
        r = jnp.dot(_unpack(o_s[c % 2]), _unpack(wo[:, cols]), preferred_element_type=F32)
        x[rows, cols] = (x[rows, cols] if it else xio[rows, cols].astype(F32)) + r

    def p_ln2(c, j):
        h2_s[j:j + LR, :] = _ln(_ln(x[pl.ds(_at(c, T, j), LR), :]))

    def p_hT(c, j):
        a = [h2_s[k * 128:(k + 1) * 128, r * DM + j * 128:r * DM + (j + 1) * 128].T for r in (0, 1) for k in (0, 1)]
        for i, v in enumerate(_lhs7(*a)):
            hS[i, j * 64:(j + 1) * 64, pl.ds(_at(c, 128), 128)] = _pack(v)

    def m1(f, s, i, c0=0, c1=NC):
        def b(k, n):
            return jnp.concatenate(
                [w1[f, c * T + k * 128:c * T + (k + 1) * 128, n * FH:(n + 1) * FH] for c in range(c0, c1)], axis=0)
        r = jnp.dot(_unpack(hS[i, :, c0 * 128:c1 * 128]), _rhs(i, b), preferred_element_type=F32)
        mb[s, i] = r + mb[s, i] if c0 else r

    def m1_0(f, i, *rng):
        m1(f, f % 2, i, *rng)

    def e1(f, s, j):
        rows = slice(j * 32, (j + 1) * 32)
        bias = b1_ref[f].astype(F32)
        u = _out4([mb[s, i, rows, :] for i in range(7)])
        g = [jax.nn.gelu(v + bias[:, (n % 2) * FH:(n % 2 + 1) * FH], approximate=True) for n, v in enumerate(u)]
        for i, v in enumerate(_lhs7(*g)):
            gS[i, j * 16:(j + 1) * 16, pl.ds(_at(f, FH), FH)] = _pack(v)

    def m2(c, i, f0=0, f1=NF):
        def b(k, n):
            return jnp.concatenate(
                [w2[c, f * FC + k * FH:f * FC + (k + 1) * FH, n * TH:(n + 1) * TH] for f in range(f0, f1)], axis=0)
        r = jnp.dot(_unpack(gS[i, :, f0 * FH:f1 * FH]), _rhs(i, b), preferred_element_type=F32)
        mb[(c + NF) % 2, i] = r + mb[(c + NF) % 2, i] if f0 else r

    def e2(it, c, j, k):
        rows, cols = slice(j * 128, (j + 1) * 128), slice(k * 128, (k + 1) * 128)
        y = _out4([mb[(c + NF) % 2, i, rows, cols] for i in range(7)])
        for n, v in enumerate(y):
            t0 = (n % 2) * TH + k * 128
            tok, ch = pl.ds(_at(c, T2, t0), 128), slice((n // 2) * DM + j * 128, (n // 2) * DM + (j + 1) * 128)
            res = x[tok, ch] + (v + b2_ref[c, :, t0:t0 + 128].astype(F32)).T
            if it:
                xio[tok, ch] = res.astype(BF16)
            else:
                x[tok, ch] = res

    def send(c):
        rows = pl.ds(_at(c, T2), T2)
        dma(xio.at[rows], out_hbm.at[rows], sems.at[7]).start()

    def each(fn, *a, n, step=1):
        return [lambda j=j: fn(*a, j) for j in range(0, n, step)]

    def l_e2(it, c):
        return [lambda j=j, k=k: e2(it, c, j, k) for k in range(TH // 128) for j in range(DM // 128)]

    def l_m(fn, c, *rng):
        return [lambda i=i: fn(c, i, *rng) for i in range(7)]

    def step(it, c, qk=1, at=1, wo_=1, ln=1, ln2=1, mm=()):
        mx = [f for t in range(3) for f in each(p_qkv, c + 1, t, n=D // MN)] * qk
        mx += each(p_wo, it, c - 1, n=D // MN) * wo_ + list(mm)
        c2 = c - 2 if isinstance(c, int) else jnp.where(c < 2, NC - 1, c - 2)
        nm = (each(p_ln2, c2, n=T, step=LR) + each(p_hT, c2, n=DM // 128)) * ln2
        nm += each(p_ln, it, c + 2, n=T, step=LR) * ln
        with jax.named_scope("y%d%d%d" % (qk, at, wo_)):
            _weave(mx, each(p_attn, c, n=T // R) * at, nm)

    def v_halo():
        for t in range(NT):
            k_s[t, 0:HALO, :] = jnp.broadcast_to(k_s[t, HALO:HALO + 1, :], (HALO, 128))
            v_s[t, 0:HALO, :] = jnp.broadcast_to(v_s[t, HALO:HALO + 1, :], (HALO, 128))

    with jax.named_scope("start"):
        cp_x0.start()
        for cp in cp_q:
            cp.start()
        cp_k.start()
        x[S - T:S, :] = jnp.zeros((T, D), F32)
        cp_x0.wait()
        _weave(each(p_ln, 0, 0, n=T, step=LR) + each(p_ln, 0, 1, n=T, step=LR))
        for p in range(KP):
            cp_q[p].wait()
            if p == 0:
                cp_v.start()
            if p == KP - 1:
                cp_o.start()
            _weave(each(prep, 0, n=NT)[p * NT // KP:(p + 1) * NT // KP])
    with jax.named_scope("start2"):
        for t, (cur, nxt) in enumerate(((cp_k, [cp_x1]), (cp_v, [cp_x2]), (cp_o, []))):
            cur.wait()
            for cp in nxt:
                cp.start()
            _weave(each(p_qkv, 0, t, n=D // MN), each(prep, t + 1, n=NT))
        cp_x1.wait()

    for it in range(2):
        v_halo()
        step(it, 0, wo_=0, ln2=0)
        if it == 0:
            cp_x2.wait()
            for cp in cp_w:
                cp.start()
        lax.fori_loop(1, NC - 1, lambda c, _, it=it: step(it, c), None)
        if it == 0:
            for cp in cp_w:
                cp.wait()
        step(it, NC - 1, qk=0, ln=0, mm=l_m(m1_0, 0, 0, NC - 3))
        step(it, NC, qk=0, at=0, ln=0)
        step(it, NC + 1, qk=0, at=0, wo_=0, ln=0, mm=l_m(m1_0, 0, NC - 3, NC - 1))
        with jax.named_scope("mix1"):
            _weave(l_m(m1_0, 0, NC - 1, NC))

            def pair(p, _):
                for s in (1, 0):
                    f = 2 * p + 2 - s
                    _weave(each(m1, f, s, n=7), each(e1, f - 1, 1 - s, n=DM // 32))
            lax.fori_loop(0, NF // 2, pair, None)
        with jax.named_scope("mix2"):
            _weave(l_m(m2, 0, 0, NF - 1), each(e1, NF - 1, (NF - 1) % 2, n=DM // 32))
            _weave(l_m(m2, 0, NF - 1, NF))

            def body(c, _, it=it):
                _weave(l_m(m2, c), l_e2(it, c - 1))
                if it:
                    send(c - 1)
            _loop(1, N2, body, U2)
        with jax.named_scope("turn"):
            if it == 0:
                _weave(each(p_ln, 1, 0, n=T, step=LR))
                _weave([f for t in range(3) for f in each(p_qkv, 0, t, n=D // MN)],
                       l_e2(0, N2 - 1) + each(p_ln, 1, 1, n=T, step=LR))
            else:
                _weave(l_e2(1, N2 - 1))
                send(N2 - 1)
    dma(xio, out_hbm, sems.at[7]).wait()


@jax.jit
def pallas_interleave_layers__sliding_local_dilated__mixer_token_mlp__prompt_kernel(
    A_x: jax.Array,
    A_wqkv: jax.Array,
    A_wo: jax.Array,
    B_x: jax.Array,
    B_w1: jax.Array,
    B_b1: jax.Array,
    B_w2: jax.Array,
    B_b2: jax.Array,
):
    del B_x
    hbm = pl.BlockSpec(memory_space=pl.ANY)
    vm = pl.BlockSpec(memory_space=pltpu.VMEM)
    out = pl.pallas_call(
        _kernel,
        out_shape=jax.ShapeDtypeStruct((S, D), A_x.dtype),
        in_specs=[hbm, hbm, hbm, hbm, vm, hbm, vm],
        out_specs=hbm,
        scratch_shapes=[
            pltpu.VMEM((S, D), BF16),
            pltpu.VMEM((4, D, D), BF16),
            pltpu.VMEM((NF, S, FC), BF16),
            pltpu.VMEM((N2, F, T2), BF16),
            pltpu.VMEM((D // 2, D), U32),
            pltpu.VMEM((D // 2, D), U32),
            pltpu.VMEM((D // 2, D), U32),
            pltpu.VMEM((D // 2, D), U32),
            pltpu.VMEM((2, H * PS, 128), F32),
            pltpu.VMEM((S, D), F32),
            pltpu.VMEM((7, DM // 2, S // 2), U32),
            pltpu.VMEM((7, DM // 2, F // 2), U32),
            pltpu.VMEM((2, 7, DM, FH), F32),
            pltpu.VMEM((2, NT, T, 128), F32),
            pltpu.VMEM((NT, S + HALO, 128), F32),
            pltpu.VMEM((NT, S + HALO, 128), F32),
            pltpu.VMEM((2, T // 2, D), U32),
            pltpu.VMEM((T, D), F32),
            pltpu.VMEM((2, T // 2, D), U32),
            pltpu.SemaphoreType.DMA((9 + KP,)),
        ],
        compiler_params=pltpu.CompilerParams(vmem_limit_bytes=126 * 1024 * 1024),
    )(A_x.reshape(S, D), A_wqkv, A_wo, B_w1, B_b1.reshape(NF, 1, FC), B_w2, B_b2.reshape(N2, 1, T2))
    return out.reshape(1, S, D)
```

```python
import math

import jax
import jax.numpy as jnp
from jax import lax
import jax.experimental.pallas as pl
import jax.experimental.pallas.tpu as pltpu

S, D, F = 2048, 1024, 3584
H, DH, W, DIL = 32, 32, 8, 2
HALO = 16
T = 256
NC = S // T
NT = D // 128
MN = 256
R = 16
LR = 32
U2 = 1
FC = 512
NF = F // FC
T2 = 512
N2 = S // T2
DM, FH, TH = D // 2, FC // 2, T2 // 2
PS = DH + 1
KP = 4
EPS = 1e-5
LOG2E = 1.4426950408889634
OFF = 1.0
F32, BF16, U32 = jnp.float32, jnp.bfloat16, jnp.uint32


def _ln(x):
    m = jnp.mean(x, axis=-1, keepdims=True)
    c = x - m
    v = jnp.mean(c * c, axis=-1, keepdims=True)
    return c * lax.rsqrt(v + EPS)


def _pack(a):
    return pltpu.bitcast(a.astype(BF16), U32)


def _unpack(a):
    return pltpu.bitcast(a, BF16)


def _lhs7(a11, a12, a21, a22):
    return (a11 + a22, a21 + a22, a11, a22, a11 + a12, a21 - a11, a12 - a22)


def _rhs(i, b):
    if i in (1, 4):
        return b(0, 0) if i == 1 else b(1, 1)
    p, q, add = {0: ((0, 0), (1, 1), True), 2: ((0, 1), (1, 1), False), 3: ((1, 0), (0, 0), False),
                 5: ((0, 0), (0, 1), True), 6: ((1, 0), (1, 1), True)}[i]
    p, q = b(*p).astype(F32), b(*q).astype(F32)
    return (p + q if add else p - q).astype(BF16)


def _out4(m):
    return (m[0] + m[3] - m[4] + m[6], m[2] + m[4], m[1] + m[3], m[0] - m[1] + m[2] + m[5])


def _weave(*streams):
    items = [((j + OFF * (s > 0)) / len(st), s, j) for s, st in enumerate(streams) for j in range(len(st))]
    for _, s, j in sorted(items):
        streams[s][j]()


def _loop(lo, hi, body, unroll):
    if unroll:
        for i in range(lo, hi):
            body(i, None)
    else:
        lax.fori_loop(lo, hi, body, None)


def _at(c, n, off=0):
    return c * n + off if isinstance(c, int) else pl.multiple_of(c * n + off, math.gcd(n, off))


def _kernel(x_hbm, wqkv_hbm, wo_hbm, w1_hbm, b1_ref, w2_hbm, b2_ref, out_hbm,
            xio, raw, w1, w2, wqT, wkT, wvT, wo, tmp, x, hS, gS, mb, q_s, k_s, v_s, h_s, h2_s, o_s, sems):
    dma = pltpu.make_async_copy
    kp = D // KP
    cp_x0 = dma(x_hbm.at[0:2 * T], xio.at[0:2 * T], sems.at[0])
    cp_x1 = dma(x_hbm.at[2 * T:3 * T], xio.at[2 * T:3 * T], sems.at[1])
    cp_x2 = dma(x_hbm.at[3 * T:S], xio.at[3 * T:S], sems.at[8])
    cp_k = dma(wqkv_hbm.at[:, D:2 * D], raw.at[1], sems.at[2])
    cp_v = dma(wqkv_hbm.at[:, 2 * D:3 * D], raw.at[2], sems.at[3])
    cp_o = dma(wo_hbm, raw.at[3], sems.at[4])
    cp_w = [dma(w1_hbm.at[:, f * FC:(f + 1) * FC], w1.at[f], sems.at[5]) for f in range(NF)]
    cp_w += [dma(w2_hbm.at[:, c * T2:(c + 1) * T2], w2.at[c], sems.at[6]) for c in range(N2)]

    def cp_q(p):
        rows = pl.ds(_at(p, kp), kp)
        return dma(wqkv_hbm.at[rows, 0:D], raw.at[0, rows], sems.at[9 + p])

    def prep(t, j, s):
        c0 = _at(j, 256, s * 128)
        a = raw[t, pl.ds(c0, 128), :].astype(F32).T if t < 3 else raw[t, :, pl.ds(c0, 128)].astype(F32)
        for h in range(H):
            tmp[s, h * PS:h * PS + DH, :] = a[h * DH:(h + 1) * DH]
        dst = (wqT, wkT, wvT, wo)[t]
        for d in range(DH):
            dst[d * H // 2:(d + 1) * H // 2, pl.ds(c0, 128)] = _pack(tmp[s, pl.ds(d, H, stride=PS), :])

    def prep2(t, j):
        prep(t, j, 0)
        prep(t, j, 1)

    def p_ln(it, c, j):
        rows = pl.ds(_at(c if isinstance(c, int) else jnp.minimum(c, NC - 1), T, j), LR)
        h_s[c % 2, j // 2:(j + LR) // 2, :] = _pack(_ln(x[rows, :] if it else xio[rows, :].astype(F32)))

    def p_qkv(c, t, j):
        w = (wqT, wkT, wvT)[t][pl.ds(_at(j, MN // 2), MN // 2), :]
        r = lax.dot_general(_unpack(h_s[c % 2]), _unpack(w), (((1,), (1,)), ((), ())), preferred_element_type=F32)
        for u in range(MN // 128):
            val, n = r[:, u * 128:(u + 1) * 128], j * (MN // 128) + u
            if t == 0:
                q_s[c % 2, n] = val
            else:
                (k_s, v_s)[t - 1][n, pl.ds(_at(c, T, HALO), T), :] = val

    def p_attn(c, j):
        r0 = _at(c, T, j * R + HALO)

        def window(ref, t):
            wide = [ref[t, pl.ds(r0 - 8 - DIL * w, R + 8), :] for w in range(W // 2)]
            return [a[8:] for a in wide] + [a[:R] for a in wide]

        lg = None
        for t in range(NT):
            q = q_s[c % 2, t, j * R:(j + 1) * R, :]
            qk = [q * k for k in window(k_s, t)]
            lg = qk if lg is None else [a + b for a, b in zip(lg, qk)]
        for w in range(W):
            a = lg[w] + pltpu.roll(lg[w], 64, 1)
            a = (a + pltpu.roll(a, 32, 1)) * (DH ** -0.5 * LOG2E)
            if isinstance(c, int) and c * T + j * R < DIL * w:
                pos = c * T + j * R + lax.broadcasted_iota(jnp.int32, (R, 128), 0)
                a = jnp.where(pos >= DIL * w, a, -1e9 * LOG2E)
            lg[w] = a
        m = lg[0]
        for w in range(1, W):
            m = jnp.maximum(m, lg[w])
        e = [jnp.exp2(a - m) for a in lg]
        den = e[0]
        for w in range(1, W):
            den = den + e[w]
        inv = 1.0 / den
        p = [a * inv for a in e]
        for t in range(NT):
            v = window(v_s, t)
            a = p[0] * v[0]
            for w in (4, 1, 5, 2, 6, 3, 7):
                a = a + p[w] * v[w]
            o_s[c % 2, j * R // 2:(j + 1) * R // 2, t * 128:(t + 1) * 128] = _pack(a)

    def p_wo(it, c, j):
        rows, cols = pl.ds(_at(c, T), T), slice(j * MN, (j + 1) * MN)
        r = jnp.dot(_unpack(o_s[c % 2]), _unpack(wo[:, cols]), preferred_element_type=F32)
        x[rows, cols] = (x[rows, cols] if it else xio[rows, cols].astype(F32)) + r

    def p_ln2(c, j):
        h2_s[j:j + LR, :] = _ln(_ln(x[pl.ds(_at(c, T, j), LR), :]))

    def p_hT(c, j):
        a = [h2_s[k * 128:(k + 1) * 128, r * DM + j * 128:r * DM + (j + 1) * 128].T for r in (0, 1) for k in (0, 1)]
        for i, v in enumerate(_lhs7(*a)):
            hS[i, j * 64:(j + 1) * 64, pl.ds(_at(c, 128), 128)] = _pack(v)

    def m1(f, s, i, c0=0, c1=NC):
        def b(k, n):
            return jnp.concatenate(
                [w1[f, c * T + k * 128:c * T + (k + 1) * 128, n * FH:(n + 1) * FH] for c in range(c0, c1)], axis=0)
        r = jnp.dot(_unpack(hS[i, :, c0 * 128:c1 * 128]), _rhs(i, b), preferred_element_type=F32)
        mb[s, i] = r + mb[s, i] if c0 else r

    def m1_0(f, i, *rng):
        m1(f, f % 2, i, *rng)

    def e1(f, s, j):
        rows = slice(j * 32, (j + 1) * 32)
        bias = b1_ref[f].astype(F32)
        u = _out4([mb[s, i, rows, :] for i in range(7)])
        g = [jax.nn.gelu(v + bias[:, (n % 2) * FH:(n % 2 + 1) * FH], approximate=True) for n, v in enumerate(u)]
        for i, v in enumerate(_lhs7(*g)):
            gS[i, j * 16:(j + 1) * 16, pl.ds(_at(f, FH), FH)] = _pack(v)

    def m2(c, i, f0=0, f1=NF):
        def b(k, n):
            return jnp.concatenate(
                [w2[c, f * FC + k * FH:f * FC + (k + 1) * FH, n * TH:(n + 1) * TH] for f in range(f0, f1)], axis=0)
        r = jnp.dot(_unpack(gS[i, :, f0 * FH:f1 * FH]), _rhs(i, b), preferred_element_type=F32)
        mb[(c + NF) % 2, i] = r + mb[(c + NF) % 2, i] if f0 else r

    def e2(it, c, j, k):
        rows, cols = slice(j * 128, (j + 1) * 128), slice(k * 128, (k + 1) * 128)
        y = _out4([mb[(c + NF) % 2, i, rows, cols] for i in range(7)])
        for n, v in enumerate(y):
            t0 = (n % 2) * TH + k * 128
            tok, ch = pl.ds(_at(c, T2, t0), 128), slice((n // 2) * DM + j * 128, (n // 2) * DM + (j + 1) * 128)
            res = x[tok, ch] + (v + b2_ref[c, :, t0:t0 + 128].astype(F32)).T
            if it:
                xio[tok, ch] = res.astype(BF16)
            else:
                x[tok, ch] = res

    def send(c):
        rows = pl.ds(_at(c, T2), T2)
        dma(xio.at[rows], out_hbm.at[rows], sems.at[7]).start()

    def each(fn, *a, n, step=1):
        return [lambda j=j: fn(*a, j) for j in range(0, n, step)]

    def l_e2(it, c):
        return [lambda j=j, k=k: e2(it, c, j, k) for k in range(TH // 128) for j in range(DM // 128)]

    def l_m(fn, c, *rng):
        return [lambda i=i: fn(c, i, *rng) for i in range(7)]

    def l_qkv(c):
        return [f for t in range(3) for f in each(p_qkv, c, t, n=D // MN)]

    def step(it, c, qk=1, at=1, wo_=1, ln=1, ln2=1, mm=()):
        mx = l_qkv(c + 1) * qk
        mx += each(p_wo, it, c - 1, n=D // MN) * wo_ + list(mm)
        c2 = c - 2 if isinstance(c, int) else jnp.where(c < 2, NC - 1, c - 2)
        nm = (each(p_ln2, c2, n=T, step=LR) + each(p_hT, c2, n=DM // 128)) * ln2
        nm += each(p_ln, it, c + 2, n=T, step=LR) * ln
        with jax.named_scope("y%d%d%d" % (qk, at, wo_)):
            _weave(mx, each(p_attn, c, n=T // R) * at, nm)

    def v_halo():
        for t in range(NT):
            k_s[t, 0:HALO, :] = jnp.broadcast_to(k_s[t, HALO:HALO + 1, :], (HALO, 128))
            v_s[t, 0:HALO, :] = jnp.broadcast_to(v_s[t, HALO:HALO + 1, :], (HALO, 128))

    with jax.named_scope("start"):
        cp_x0.start()
        for p in range(KP):
            cp_q(p).start()
        cp_k.start()
        x[S - T:S, :] = jnp.zeros((T, D), F32)
        cp_x0.wait()
        lax.fori_loop(0, 2, lambda c, _: _weave(each(p_ln, 0, c, n=T, step=LR)), None)
        cp_v.start()

        def first(p, _):
            cp_q(p).wait()
            prep2(0, p)
        lax.fori_loop(0, KP, first, None)
        cp_o.start()
    with jax.named_scope("start2"):
        for t, (cur, nxt) in enumerate(((cp_k, [cp_x1]), (cp_v, [cp_x2]), (cp_o, []))):
            cur.wait()
            for cp in nxt:
                cp.start()

            def piece(j, _, t=t):
                p_qkv(0, t, j)
                prep2(t + 1, j)
            lax.fori_loop(0, D // MN, piece, None)
        cp_x1.wait()

    for it in range(2):
        v_halo()
        step(it, 0, wo_=0, ln2=0)
        if it == 0:
            cp_x2.wait()
            for cp in cp_w:
                cp.start()
        lax.fori_loop(1, NC - 1, lambda c, _, it=it: step(it, c), None)
        if it == 0:
            for cp in cp_w:
                cp.wait()
        step(it, NC - 1, qk=0, ln=0, mm=l_m(m1_0, 0, 0, NC - 3))
        step(it, NC, qk=0, at=0, ln=0)
        step(it, NC + 1, qk=0, at=0, wo_=0, ln=0, mm=l_m(m1_0, 0, NC - 3, NC - 1))
        with jax.named_scope("mix1"):
            _weave(l_m(m1_0, 0, NC - 1, NC))

            def pair(p, _):
                for s in (1, 0):
                    f = 2 * p + 2 - s
                    _weave(each(m1, f, s, n=7), each(e1, f - 1, 1 - s, n=DM // 32))
            lax.fori_loop(0, NF // 2, pair, None)
        with jax.named_scope("mix2"):
            _weave(l_m(m2, 0, 0, NF - 1), each(e1, NF - 1, (NF - 1) % 2, n=DM // 32))
            _weave(l_m(m2, 0, NF - 1, NF))

            def body(c, _, it=it):
                _weave(l_m(m2, c), l_e2(it, c - 1))
                if it:
                    send(c - 1)
            _loop(1, N2, body, U2)
        with jax.named_scope("turn"):
            if it == 0:
                _weave(each(p_ln, 1, 0, n=T, step=LR))
                _weave(l_qkv(0),
                       l_e2(0, N2 - 1) + each(p_ln, 1, 1, n=T, step=LR))
            else:
                _weave(l_e2(1, N2 - 1))
                send(N2 - 1)
    dma(xio, out_hbm, sems.at[7]).wait()


@jax.jit
def pallas_interleave_layers__sliding_local_dilated__mixer_token_mlp__prompt_kernel(
    A_x: jax.Array,
    A_wqkv: jax.Array,
    A_wo: jax.Array,
    B_x: jax.Array,
    B_w1: jax.Array,
    B_b1: jax.Array,
    B_w2: jax.Array,
    B_b2: jax.Array,
):
    del B_x
    hbm = pl.BlockSpec(memory_space=pl.ANY)
    vm = pl.BlockSpec(memory_space=pltpu.VMEM)
    out = pl.pallas_call(
        _kernel,
        out_shape=jax.ShapeDtypeStruct((S, D), A_x.dtype),
        in_specs=[hbm, hbm, hbm, hbm, vm, hbm, vm],
        out_specs=hbm,
        scratch_shapes=[
            pltpu.VMEM((S, D), BF16),
            pltpu.VMEM((4, D, D), BF16),
            pltpu.VMEM((NF, S, FC), BF16),
            pltpu.VMEM((N2, F, T2), BF16),
            pltpu.VMEM((D // 2, D), U32),
            pltpu.VMEM((D // 2, D), U32),
            pltpu.VMEM((D // 2, D), U32),
            pltpu.VMEM((D // 2, D), U32),
            pltpu.VMEM((2, H * PS, 128), F32),
            pltpu.VMEM((S, D), F32),
            pltpu.VMEM((7, DM // 2, S // 2), U32),
            pltpu.VMEM((7, DM // 2, F // 2), U32),
            pltpu.VMEM((2, 7, DM, FH), F32),
            pltpu.VMEM((2, NT, T, 128), F32),
            pltpu.VMEM((NT, S + HALO, 128), F32),
            pltpu.VMEM((NT, S + HALO, 128), F32),
            pltpu.VMEM((2, T // 2, D), U32),
            pltpu.VMEM((T, D), F32),
            pltpu.VMEM((2, T // 2, D), U32),
            pltpu.SemaphoreType.DMA((9 + KP,)),
        ],
        compiler_params=pltpu.CompilerParams(vmem_limit_bytes=126 * 1024 * 1024),
    )(A_x.reshape(S, D), A_wqkv, A_wo, B_w1, B_b1.reshape(NF, 1, FC), B_w2, B_b2.reshape(N2, 1, T2))
    return out.reshape(1, S, D)
```
